```python
import os as _os
_os.environ.setdefault("JAX_PLATFORMS", "cpu")
import jax
import jax.numpy as jnp

def _softmax(x, axis=-1):
    return jax.nn.softmax(x, axis=axis)
def _gelu(x):
    return jax.nn.gelu(x, approximate=True)
def _silu(x):
    return jax.nn.silu(x)
def _sigmoid(x):
    return jax.nn.sigmoid(x)
def _layernorm(x, axis=-1, eps=1e-5):
    m = jnp.mean(x, axis=axis, keepdims=True)
    v = jnp.var(x, axis=axis, keepdims=True)
    return (x - m) / jnp.sqrt(v + eps)
def _scatter_add(tgt, idx, src, axis=0):
    return tgt.at[idx].add(src)
def _segment_sum(src, seg, n):
    return jax.ops.segment_sum(src, seg, n)
class _Rng:
    def __init__(self, key):
        self._k = key
    def _next(self):
        self._k, sub = jax.random.split(self._k)
        return sub
    def normal(self, shape):
        return jax.random.normal(self._next(), shape, dtype=jnp.bfloat16)
    def randint(self, lo, hi, shape):
        return jax.random.randint(self._next(), shape, lo, hi, dtype=jnp.int32)
    def uniform(self, shape, lo=0.0, hi=1.0):
        return jax.random.uniform(self._next(), shape, jnp.bfloat16, lo, hi)
    def permutation(self, n):
        return jax.random.permutation(self._next(), n)


kernel_name = 'sequential_preLN__sliding_block__dense_activation_gelu__prompt'

def setup_inputs():
    _rng = _Rng(jax.random.key(int.from_bytes(__import__("os").urandom(4), "little")))
    _w = (lambda a: (lambda t: t.astype(jnp.bfloat16) if jnp.issubdtype(t.dtype, jnp.floating) else t)(jnp.asarray(a)))
    def _A_setup():
        B, S, D = 1, 2048, 640
        return {
            "x": _w((lambda *s: _rng.normal(s) * 0.05)(B, S, D)),
            "wqkv": _w((lambda *s: _rng.normal(s) * 0.05)(D, 3 * D)),
            "wo": _w((lambda *s: _rng.normal(s) * 0.05)(D, D)),
        }
    _A_in = _A_setup()

    def _B_setup():
        B, S, D, F = 1, 2048, 640, 1536
        return {
            "x": _w((lambda *s: _rng.normal(s) * 0.05)(B, S, D)),
            "w1": _w((lambda *s: _rng.normal(s) * 0.8)(D, F) * (D ** -0.5)),
            "b1": _w((lambda *s: _rng.normal(s) * 0.8)(F) * 0.01),
            "w2": _w((lambda *s: _rng.normal(s) * 0.8)(F, D) * (F ** -0.5)),
            "b2": _w((lambda *s: _rng.normal(s) * 0.05)(D) * 0.01),
        }
    _B_in = _B_setup()

    return {
        "A_x": _A_in["x"],
        "A_wqkv": _A_in["wqkv"],
        "A_wo": _A_in["wo"],
        "B_x": _B_in["x"],
        "B_w1": _B_in["w1"],
        "B_b1": _B_in["b1"],
        "B_w2": _B_in["w2"],
        "B_b2": _B_in["b2"],
    }

def reference(A_x, A_wqkv, A_wo, B_x, B_w1, B_b1, B_w2, B_b2):
    def _A_ref(x, wqkv, wo):
        B, S, D = x.shape
        H = 32; Dh = D // H; W = 256
        qkv = (lambda x, *d: x.transpose(*d))((x @ wqkv).reshape(B, S, 3, H, Dh), 2, 0, 3, 1, 4)
        q, k, v = qkv[0], qkv[1], qkv[2]
        scores = jnp.einsum("bhqd,bhkd->bhqk", q, k) * (Dh ** -0.5)
        idx = jnp.arange(S)
        mask = (idx[:, None] - idx[None, :] >= 0) & (idx[:, None] - idx[None, :] < W)
        scores = jnp.where(mask[None, None], scores, -1e9)
        p = _softmax(scores, axis=-1)
        o = jnp.einsum("bhqk,bhkd->bhqd", p, v)
        return (lambda x, *d: x.transpose(*d))(o, 0, 2, 1, 3).reshape(B, S, D) @ wo

    def _B_ref(x, w1, b1, w2, b2):
        h = jnp.einsum("bsd,df->bsf", x, w1) + b1
        h = _gelu(h)
        return jnp.einsum("bsf,fd->bsd", h, w2) + b2

    x = A_x
    h = x + _A_ref(_layernorm(x, axis=-1), A_wqkv, A_wo)
    h2 = h + _B_ref(_layernorm(h, axis=-1), B_w1, B_b1, B_w2, B_b2)
    return h2
```

```python
import math

import jax
import jax.numpy as jnp
from jax import lax
from jax.experimental import pallas as pl
from jax.experimental.pallas import tpu as pltpu

S = 2048
D = 640
H = 32
DH = 20
F = 1536
TQ = 256
NSTEP = S // TQ
NQUAD = 8
QW = 4 * DH
QUAD_WIN = (0, 1, 2, 3, 5, 6, 7, 8)
VROWS = 32
NEG = -1e30
EPS = 1e-5
QSCALE = (DH ** -0.5) * math.log2(math.e)
NT = (((1,), (1,)), ((), ()))
BF = jnp.bfloat16
F32 = jnp.float32
F1C = 128
F2R = 128
TAILF = 2
KCH = (128, 256, 256)
KOFF = (0, 128, 384, 640)
HSEQ = ('q0 q1 q2 q3 q4 q5 W q6 q7 P P Va P a0 a1 Vb a2 a3 P a4 a5 U0 a6 a7 b0 U1 b1 b2 P b3 b4 '
        'U2 b5 O0 b6 b7 P O1 P P P P U3 X')


def _ln(x):
    m = jnp.mean(x, axis=-1, keepdims=True)
    xc = x - m
    v = jnp.mean(xc * xc, axis=-1, keepdims=True)
    return xc * lax.rsqrt(v + EPS)


def _gelu(x):
    c = math.sqrt(2.0 / math.pi)
    inner = x * (c + (c * 0.044715) * (x * x))
    hx = 0.5 * x
    return hx + hx * jnp.tanh(inner)


def _window(chunks, w, lane):
    if w % 2 == 0:
        return chunks[w // 2]
    return jnp.where(lane >= 64, chunks[w // 2], chunks[w // 2 + 1])


def _colmax(a):
    return jnp.max(a.reshape(a.shape[0] // 8, 8, 128), axis=0)


def _split128(a):
    return [a[:, c * 128:(c + 1) * 128] for c in range(a.shape[1] // 128)]


def _kernel(x_hbm, wqkv_hbm, wo_hbm, w1_hbm, b1_hbm, w2_hbm, b2_hbm, o_hbm,
            x_scr, o_scr, wvt_scr, q_scr, k_scr, vt_scr, att_scr, hn_scr, s_scr, m_scr, zt_scr,
            wqkv_ref, wo_ref, w1_ref, w2_ref, b1_ref, b2_ref, sems):
    i = pl.program_id(0)

    cp_x0 = pltpu.make_async_copy(x_hbm.at[0:TQ], x_scr.at[0:TQ], sems.at[2])
    cp_x1 = pltpu.make_async_copy(x_hbm.at[TQ:2 * TQ], x_scr.at[TQ:2 * TQ], sems.at[0])
    cp_xr = pltpu.make_async_copy(x_hbm.at[2 * TQ:S], x_scr.at[2 * TQ:S], sems.at[2])

    def cp_qk(c):
        r = pl.ds(pl.multiple_of((i >> 20) * 128 + KOFF[c], 128), KCH[c])
        return pltpu.make_async_copy(wqkv_hbm.at[KOFF[c]:KOFF[c + 1], 0:2 * D],
                                     wqkv_ref.at[r, 0:2 * D], sems.at[c])

    def cp_o(n):
        r = pl.ds(n * TQ, TQ) if isinstance(n, int) else pl.ds(pl.multiple_of(n * TQ, TQ), TQ)
        return pltpu.make_async_copy(o_scr.at[r], o_hbm.at[r], sems.at[3])

    def cp_ol(r, c0, c1):
        rs = pl.ds((NSTEP - 1) * TQ + r * (TQ // 2), TQ // 2)
        return pltpu.make_async_copy(o_scr.at[rs, c0:c1], o_hbm.at[rs, c0:c1], sems.at[3])

    cp_wv = pltpu.make_async_copy(wqkv_hbm.at[:, 2 * D:3 * D], wqkv_ref.at[:, 2 * D:3 * D], sems.at[0])
    cp_wo = pltpu.make_async_copy(wo_hbm, wo_ref, sems.at[0])
    cp_b1 = pltpu.make_async_copy(b1_hbm, b1_ref, sems.at[0])
    cp_b2 = pltpu.make_async_copy(b2_hbm, b2_ref, sems.at[0])
    cp_w1 = pltpu.make_async_copy(w1_hbm, w1_ref, sems.at[1])
    cp_w2 = pltpu.make_async_copy(w2_hbm, w2_ref, sems.at[1])

    lane32 = lax.broadcasted_iota(jnp.int32, (32, 128), 1)
    row32 = lax.broadcasted_iota(jnp.int32, (32, 128), 0)
    lane128 = lax.broadcasted_iota(jnp.int32, (128, 128), 1)
    row128 = lax.broadcasted_iota(jnp.int32, (128, 128), 0)

    def ln1(row0):
        return _ln(x_scr[pl.ds(row0, TQ), :].astype(F32)).astype(BF)

    def store_qk(chunks, row0, qs):
        qc = [c * QSCALE for c in chunks[0:5]]
        kc = chunks[5:10]
        lane = lax.broadcasted_iota(jnp.int32, (TQ, 128), 1)
        for g in range(NQUAD):
            q_scr[qs, g] = _window(qc, QUAD_WIN[g], lane)
            k_scr[g, pl.ds(row0, TQ), :] = _window(kc, QUAD_WIN[g], lane).astype(BF)

    def v_proj(xn, row0, h0, h1):
        f0 = h0 * DH
        vt = lax.dot_general(wvt_scr[f0:h1 * DH, :], xn, NT, preferred_element_type=F32)
        ones = jnp.ones((8, TQ), F32)
        for h in range(h0, h1):
            r0 = (h // 2) * 40 + (h % 2) * 16 - f0
            blk = jnp.concatenate([vt[r0:r0 + 24, :], ones], axis=0)
            vt_scr[h, :, pl.ds(row0, TQ)] = blk.astype(BF)

    def pieces(qs, g, qoff):
        out = {}
        for j in range(4):
            msk = ((lane32 - (g * QW + j * DH) % 128) & 127) < DH
            for t in range(4):
                out[(j, t)] = jnp.where(msk, q_scr[qs, g, qoff + 32 * t:qoff + 32 * t + 32, :], 0.0)
        return out

    def head_tiles(pc):
        return jnp.concatenate([pc[(j, s ^ j)] for j in range(4) for s in range(4)], axis=0).astype(BF)

    def qk_phase(g, jb, base, sl):
        pc = pieces(0, g, jb * 128)
        tri32 = row32 <= (lane32 & 31)
        klo = k_scr[g, pl.ds(base - 256, 128), :]
        kmid = k_scr[g, pl.ds(base - 128, 128), :]
        khi = k_scr[g, pl.ds(base, 128), :]
        es = []
        for t in range(4):
            lhs = jnp.concatenate([klo[32 * t:128], khi[0:32 * (t + 1)]], axis=0)
            ct = jnp.concatenate([pc[(s ^ t, t)] for s in range(4)], axis=0).astype(BF)
            r = lax.dot_general(lhs, ct, NT, preferred_element_type=F32)
            nlo = 128 - 32 * t
            ch = []
            for c in range(4):
                if c > t:
                    ch.append(r[32 * (c - t):32 * (c - t) + 32])
                elif c < t:
                    ch.append(r[nlo + 32 * c:nlo + 32 * c + 32])
                else:
                    ch.append(jnp.where(tri32, r[nlo + 32 * t:nlo + 32 * t + 32], r[0:32]))
            es.append(jnp.concatenate(ch, axis=0))
        b64 = (lane128 & 64) != 0
        b32 = (lane128 & 32) != 0
        ys = [jnp.where(b64, es[t ^ 2], es[t]) for t in range(4)]
        gs = [jnp.where(b32, ys[j ^ 1], ys[j]) for j in range(4)]
        mids = lax.dot_general(kmid, head_tiles(pc), NT, preferred_element_type=F32)
        for j in range(4):
            mid = mids[:, 128 * j:128 * (j + 1)]
            m = jnp.max(jnp.maximum(_colmax(gs[j]), _colmax(mid)), axis=0, keepdims=True)
            s_scr[sl, j, 0:128, :] = gs[j]
            s_scr[sl, j, 128:256, :] = mid
            m_scr[sl, j] = jnp.broadcast_to(m, (8, 128))

    def normalize(r):
        inv = 1.0 / r[24:32]
        return r[0:24] * jnp.concatenate([inv] * 3, axis=0)

    def finish_block(jb):
        qoff = jb * 128
        feat = lax.broadcasted_iota(jnp.int32, (32, D), 1)
        hq = ((feat * 3277) >> 16) & 3
        hb1 = (hq & 2) != 0
        hb0 = (hq & 1) != 0
        t = zt_scr[:, qoff:qoff + 128].T
        ts = [t[32 * u:32 * u + 32] for u in range(4)]
        us = [jnp.where(hb1, ts[u ^ 2], ts[u]) for u in range(4)]
        for u in range(4):
            o = jnp.where(hb0, us[u ^ 1], us[u])
            att_scr[qoff + 32 * u:qoff + 32 * u + 32, :] = o.astype(BF)

    def finish_heads(g, jb, rs):
        qoff = jb * 128
        row8 = lax.broadcasted_iota(jnp.int32, (8, 128), 0)
        for p in range(2):
            re_, ro = rs[2 * p], rs[2 * p + 1]
            z = jnp.concatenate([re_[0:16], jnp.where(row8 < 4, re_[16:24], ro[0:8]), ro[8:24]], axis=0)
            r0 = g * QW + p * 40
            zt_scr[r0:r0 + 40, qoff:qoff + 128] = z
        if g == NQUAD - 1:
            finish_block(jb)

    def pv_phase(g, jb, base, sl):
        rs = []
        for j in range(4):
            m = m_scr[sl, j][0:1, :]
            pg = jnp.exp2(s_scr[sl, j, 0:128, :] - m)
            pm = jnp.exp2(s_scr[sl, j, 128:256, :] - m)
            mhi = row128 <= (lane128 ^ (32 * j))
            phi = jnp.where(mhi, pg, 0.0)
            plo = jnp.where(mhi, 0.0, pg)
            pf = jnp.concatenate([plo, pm, phi], axis=0).astype(BF)
            vv = vt_scr[4 * g + j, :, pl.ds(base - 256, 384)]
            rs.append(normalize(jnp.dot(vv, pf, preferred_element_type=F32)))
        finish_heads(g, jb, rs)

    def qk_phase0(g, jb):
        qoff = jb * 128
        nk = qoff + 128
        sl = jb * NQUAD + g
        st = lax.dot_general(k_scr[g, 0:nk, :], head_tiles(pieces(1, g, qoff)), NT,
                             preferred_element_type=F32)
        for j in range(4):
            sj = st[:, 128 * j:128 * (j + 1)]
            mhi = row128 <= (lane128 ^ (32 * j))
            hi = jnp.where(mhi, sj[nk - 128:nk], NEG)
            m8 = _colmax(hi)
            s_scr[sl, j, 0:128, :] = hi
            if nk > 128:
                m8 = jnp.maximum(m8, _colmax(sj[0:128]))
                s_scr[sl, j, 128:256, :] = sj[0:128]
            m = jnp.max(m8, axis=0, keepdims=True)
            m_scr[sl, j] = jnp.broadcast_to(m, (8, 128))

    def pv_phase0(g, jb):
        nk = jb * 128 + 128
        sl = jb * NQUAD + g
        rs = []
        for j in range(4):
            m = m_scr[sl, j][0:1, :]
            phi = jnp.exp2(s_scr[sl, j, 0:128, :] - m)
            if nk > 128:
                pm = jnp.exp2(s_scr[sl, j, 128:256, :] - m)
                pf = jnp.concatenate([pm, phi], axis=0).astype(BF)
            else:
                pf = phi.astype(BF)
            rs.append(normalize(jnp.dot(vt_scr[4 * g + j, :, 0:nk], pf, preferred_element_type=F32)))
        finish_heads(g, jb, rs)

    work = [(g, jb) for jb in range(TQ // 128) for g in range(NQUAD)]

    def attention(row0, fillers):
        def base_of(jb):
            if isinstance(row0, int):
                return row0 + jb * 128
            return pl.multiple_of(row0 + jb * 128, 128)

        def do_qk(n):
            g, jb = work[n]
            qk_phase(g, jb, base_of(jb), n % 2)

        nw = len(work)
        nf = len(fillers) - TAILF
        fi = 0
        do_qk(0)
        for n in range(nw):
            if n + 1 < nw:
                do_qk(n + 1)
            while fi < ((n + 1) * nf) // nw:
                fillers[fi]()
                fi += 1
            g, jb = work[n]
            pv_phase(g, jb, base_of(jb), n % 2)
        while fi < len(fillers):
            fillers[fi]()
            fi += 1

    def out_proj(prow0, r0, nr):
        xp = x_scr[pl.ds(prow0 + r0, nr), :].astype(F32)
        return xp + jnp.dot(att_scr[r0:r0 + nr, :], wo_ref[...], preferred_element_type=F32)

    def ffn_fillers(h, hn, prow0, r0, nr):
        gl = []
        fl = []
        bias = {}

        def f1(c):
            def run():
                if c == 0:
                    bias['b1'] = b1_ref[...].astype(F32).reshape(1, F)
                u = jnp.dot(hn, w1_ref[:, c * F1C:(c + 1) * F1C], preferred_element_type=F32)
                u = u + bias['b1'][:, c * F1C:(c + 1) * F1C]
                gl.append(_gelu(u).astype(BF))
            return run

        def f2(n, r):
            def run():
                if n == 0 and r == 0:
                    bias['b2'] = b2_ref[...].astype(F32).reshape(1, D)
                rows = slice(r * F2R, (r + 1) * F2R)
                cols = slice(n * 128, (n + 1) * 128)
                y = h[rows, cols] + bias['b2'][:, cols]
                for c in range(F // F1C):
                    y = y + jnp.dot(gl[c][rows], w2_ref[c * F1C:(c + 1) * F1C, cols],
                                    preferred_element_type=F32)
                o_scr[pl.ds(prow0 + (r0 + r * F2R), F2R), cols] = y.astype(BF)
            return run

        for c in range(F // F1C):
            fl.append(f1(c))
        for r in range(nr // F2R):
            for n in range(D // 128):
                fl.append(f2(n, r))
        return fl

    @pl.when(i == 0)
    def _head():
        cp_x0.start()
        cp_qk(0).start()
        cp_qk(1).start()
        cp_x0.wait()
        xn0 = ln1(0)
        qk = None
        for c in range(3):
            cp_qk(c).wait()
            if c == 0:
                cp_qk(2).start()
            elif c == 1:
                cp_x1.start()
                cp_wv.start()
            else:
                cp_wo.start()
                cp_b1.start()
                cp_b2.start()
            wc = wqkv_ref[KOFF[c]:KOFF[c + 1], 0:2 * D]
            if c == 0:
                part = jnp.concatenate(
                    [jnp.dot(xn0[r:r + 128, KOFF[c]:KOFF[c + 1]], wc, preferred_element_type=F32)
                     for r in range(0, TQ, 128)], axis=0)
            else:
                part = jnp.dot(xn0[:, KOFF[c]:KOFF[c + 1]], wc, preferred_element_type=F32)
            qk = part if qk is None else qk + part
        store_qk(_split128(qk), 0, 1)
        for g in range(NQUAD):
            qk_phase0(g, 0)
        parts = []
        st = {}
        for op in HSEQ.split():
            if op == 'P':
                c = len(parts)
                parts.append(jnp.dot(st['xn1'], wqkv_ref[:, c * 128:(c + 1) * 128],
                                     preferred_element_type=F32))
                if c == 9:
                    store_qk(parts, TQ, 0)
            elif op == 'W':
                cp_x1.wait()
                cp_wv.wait()
                cp_wo.wait()
                cp_b1.wait()
                cp_b2.wait()
                cp_w1.start()
                cp_w2.start()
                wvt_scr[...] = wqkv_ref[:, 2 * D:3 * D].astype(F32).T.astype(BF)
                st['xn1'] = ln1(TQ)
            elif op == 'X':
                cp_w1.wait()
                cp_w2.wait()
                cp_xr.start()
            elif op == 'Va':
                v_proj(xn0, 0, 0, H // 2)
            elif op == 'Vb':
                v_proj(xn0, 0, H // 2, H)
            elif op[0] == 'U':
                u = int(op[1])
                v_proj(st['xn1'], TQ, u * 8, u * 8 + 8)
            elif op[0] == 'O':
                r = int(op[1])
                hh = out_proj(0, r * 128, 128)
                st['h%d' % r] = hh
                hn_scr[r * 128:(r + 1) * 128, :] = _ln(hh).astype(BF)
            elif op[0] == 'q':
                qk_phase0(int(op[1]), 1)
            elif op[0] == 'a':
                pv_phase0(int(op[1]), 0)
            elif op[0] == 'b':
                pv_phase0(int(op[1]), 1)
        h = jnp.concatenate([st['h0'], st['h1']], axis=0)
        attention(TQ, ffn_fillers(h, hn_scr[...], 0, 0, TQ))
        cp_o(0).start()
        cp_xr.wait()

    @pl.when(jnp.logical_and(i > 0, i < NSTEP - 1))
    def _main():
        row0 = pl.multiple_of((i + 1) * TQ, TQ)
        h = out_proj(row0 - TQ, 0, TQ)
        hn = _ln(h).astype(BF)
        xn = ln1(row0)
        qk = jnp.dot(xn, wqkv_ref[:, 0:2 * D], preferred_element_type=F32)
        store_qk(_split128(qk), row0, 0)
        v_proj(xn, row0, 0, H)
        attention(row0, ffn_fillers(h, hn, row0 - TQ, 0, TQ))
        cp_o(i).start()

    @pl.when(i == NSTEP - 1)
    def _last():
        prow0 = (NSTEP - 1) * TQ
        hr = TQ // 2
        ha = out_proj(prow0, 0, hr)
        hna = _ln(ha).astype(BF)
        hb = out_proj(prow0, hr, hr)
        hnb = _ln(hb).astype(BF)
        fa = ffn_fillers(ha, hna, prow0, 0, hr)
        fb = ffn_fillers(hb, hnb, prow0, hr, hr)
        n1 = F // F1C
        for f in fa[:n1] + fb[:n1] + fa[n1:] + fb[n1:n1 + 2]:
            f()
        cp_ol(0, 0, D).start()
        for f in fb[n1 + 2:n1 + 4]:
            f()
        cp_ol(1, 0, 256).start()
        for f in fb[n1 + 4:]:
            f()
        cp_ol(1, 256, D).start()
        for n in range(NSTEP - 1):
            cp_o(n).wait()
        cp_ol(0, 0, D).wait()
        cp_ol(1, 0, 256).wait()
        cp_ol(1, 256, D).wait()


@jax.jit
def pallas_sequential_preLN__sliding_block__dense_activation_gelu__prompt_kernel(
    A_x: jax.Array,
    A_wqkv: jax.Array,
    A_wo: jax.Array,
    B_x: jax.Array,
    B_w1: jax.Array,
    B_b1: jax.Array,
    B_w2: jax.Array,
    B_b2: jax.Array,
):
    del B_x
    anyspec = pl.BlockSpec(memory_space=pl.ANY)
    out = pl.pallas_call(
        _kernel,
        grid=(NSTEP,),
        in_specs=[anyspec] * 7,
        out_specs=anyspec,
        out_shape=jax.ShapeDtypeStruct((S, D), BF),
        scratch_shapes=[
            pltpu.VMEM((S, D), BF),
            pltpu.VMEM((S, D), BF),
            pltpu.VMEM((D, D), BF),
            pltpu.VMEM((2, NQUAD, TQ, 128), F32),
            pltpu.VMEM((NQUAD, S, 128), BF),
            pltpu.VMEM((H, VROWS, S), BF),
            pltpu.VMEM((TQ, D), BF),
            pltpu.VMEM((TQ, D), BF),
            pltpu.VMEM((2 * NQUAD, 4, 256, 128), F32),
            pltpu.VMEM((2 * NQUAD, 4, 8, 128), F32),
            pltpu.VMEM((D, TQ), F32),
            pltpu.VMEM((D, 3 * D), BF),
            pltpu.VMEM((D, D), BF),
            pltpu.VMEM((D, F), BF),
            pltpu.VMEM((F, D), BF),
            pltpu.VMEM((F,), BF),
            pltpu.VMEM((D,), BF),
            pltpu.SemaphoreType.DMA((4,)),
        ],
        compiler_params=pltpu.CompilerParams(
            dimension_semantics=("arbitrary",),
            vmem_limit_bytes=100 * 1024 * 1024),
    )(A_x.reshape(S, D), A_wqkv, A_wo, B_w1, B_b1, B_w2, B_b2)
    return out.reshape(1, S, D)
```

```python
import math

import jax
import jax.numpy as jnp
from jax import lax
from jax.experimental import pallas as pl
from jax.experimental.pallas import tpu as pltpu

S = 2048
D = 640
H = 32
DH = 20
F = 1536
TQ = 256
NSTEP = S // TQ
NQUAD = 8
QW = 4 * DH
QUAD_WIN = (0, 1, 2, 3, 5, 6, 7, 8)
VROWS = 32
NEG = -1e30
EPS = 1e-5
QSCALE = (DH ** -0.5) * math.log2(math.e)
NT = (((1,), (1,)), ((), ()))
BF = jnp.bfloat16
F32 = jnp.float32
F1C = 128
F2R = 128
TAILF = 2
KCH = (128, 256, 256)
KOFF = (0, 128, 384, 640)
HSEQ = ('q0 W q1 q2 q3 P P q4 Va P a0 a1 Vb a2 a3 P a4 a5 q5 a6 a7 P b0 q6 b1 P b2 q7 b3 P b4 P b5 '
        'P b6 P b7 U0 K0 K1 U1 Z0 K2 U2 Z1 K3 X O0 Z2 O1 K4 U3 Z3 K5 Z4 K6 F Z5 K7 F F Z6 K8 F F Z7 '
        'K9 F F Z8 K10 F F Z9 K11 F F Z10 K12 F F Z11 K13 F F Z12 K14 F F Z13 K15 F F Z14 F Z15 F F')


def _ln(x):
    m = jnp.mean(x, axis=-1, keepdims=True)
    xc = x - m
    v = jnp.mean(xc * xc, axis=-1, keepdims=True)
    return xc * lax.rsqrt(v + EPS)


def _gelu(x):
    c = math.sqrt(2.0 / math.pi)
    inner = x * (c + (c * 0.044715) * (x * x))
    hx = 0.5 * x
    return hx + hx * jnp.tanh(inner)


def _window(chunks, w, lane):
    if w % 2 == 0:
        return chunks[w // 2]
    return jnp.where(lane >= 64, chunks[w // 2], chunks[w // 2 + 1])


def _colmax(a):
    return jnp.max(a.reshape(a.shape[0] // 8, 8, 128), axis=0)


def _split128(a):
    return [a[:, c * 128:(c + 1) * 128] for c in range(a.shape[1] // 128)]


def _kernel(x_hbm, wqkv_hbm, wo_hbm, w1_hbm, b1_hbm, w2_hbm, b2_hbm, o_hbm,
            x_scr, o_scr, wvt_scr, q_scr, k_scr, vt_scr, att_scr, s_scr, m_scr, zt_scr,
            wqkv_ref, wo_ref, w1_ref, w2_ref, b1_ref, b2_ref, sems):
    i = pl.program_id(0)

    cp_x0 = pltpu.make_async_copy(x_hbm.at[0:TQ], x_scr.at[0:TQ], sems.at[2])
    cp_x1 = pltpu.make_async_copy(x_hbm.at[TQ:2 * TQ], x_scr.at[TQ:2 * TQ], sems.at[0])
    cp_xr = pltpu.make_async_copy(x_hbm.at[2 * TQ:S], x_scr.at[2 * TQ:S], sems.at[2])

    def cp_qk(c):
        r = pl.ds(pl.multiple_of((i >> 20) * 128 + KOFF[c], 128), KCH[c])
        return pltpu.make_async_copy(wqkv_hbm.at[KOFF[c]:KOFF[c + 1], 0:2 * D],
                                     wqkv_ref.at[r, 0:2 * D], sems.at[c])

    def cp_o(n):
        r = pl.ds(n * TQ, TQ) if isinstance(n, int) else pl.ds(pl.multiple_of(n * TQ, TQ), TQ)
        return pltpu.make_async_copy(o_scr.at[r], o_hbm.at[r], sems.at[3])

    def cp_ol(r, c0, c1):
        rs = pl.ds((NSTEP - 1) * TQ + r * (TQ // 2), TQ // 2)
        return pltpu.make_async_copy(o_scr.at[rs, c0:c1], o_hbm.at[rs, c0:c1], sems.at[3])

    cp_wv = pltpu.make_async_copy(wqkv_hbm.at[:, 2 * D:3 * D], wqkv_ref.at[:, 2 * D:3 * D], sems.at[0])
    cp_wo = pltpu.make_async_copy(wo_hbm, wo_ref, sems.at[1])
    cp_b1 = pltpu.make_async_copy(b1_hbm, b1_ref, sems.at[1])
    cp_b2 = pltpu.make_async_copy(b2_hbm, b2_ref, sems.at[1])
    cp_w1 = pltpu.make_async_copy(w1_hbm, w1_ref, sems.at[1])
    cp_w2 = pltpu.make_async_copy(w2_hbm, w2_ref, sems.at[1])

    lane32 = lax.broadcasted_iota(jnp.int32, (32, 128), 1)
    row32 = lax.broadcasted_iota(jnp.int32, (32, 128), 0)
    lane128 = lax.broadcasted_iota(jnp.int32, (128, 128), 1)
    row128 = lax.broadcasted_iota(jnp.int32, (128, 128), 0)

    def ln1(row0):
        return _ln(x_scr[pl.ds(row0, TQ), :].astype(F32)).astype(BF)

    def store_qk(chunks, row0, qs):
        qc = [c * QSCALE for c in chunks[0:5]]
        kc = chunks[5:10]
        lane = lax.broadcasted_iota(jnp.int32, (TQ, 128), 1)
        for g in range(NQUAD):
            q_scr[qs, g] = _window(qc, QUAD_WIN[g], lane)
            k_scr[g, pl.ds(row0, TQ), :] = _window(kc, QUAD_WIN[g], lane).astype(BF)

    def v_proj(xn, row0, h0, h1):
        f0 = h0 * DH
        vt = lax.dot_general(wvt_scr[f0:h1 * DH, :], xn, NT, preferred_element_type=F32)
        ones = jnp.ones((8, TQ), F32)
        for h in range(h0, h1):
            r0 = (h // 2) * 40 + (h % 2) * 16 - f0
            blk = jnp.concatenate([vt[r0:r0 + 24, :], ones], axis=0)
            vt_scr[h, :, pl.ds(row0, TQ)] = blk.astype(BF)

    def pieces(qs, g, qoff):
        out = {}
        for j in range(4):
            msk = ((lane32 - (g * QW + j * DH) % 128) & 127) < DH
            for t in range(4):
                out[(j, t)] = jnp.where(msk, q_scr[qs, g, qoff + 32 * t:qoff + 32 * t + 32, :], 0.0)
        return out

    def head_tiles(pc):
        return jnp.concatenate([pc[(j, s ^ j)] for j in range(4) for s in range(4)], axis=0).astype(BF)

    def group_tile(pc, t):
        return jnp.concatenate([pc[(s ^ t, t)] for s in range(4)], axis=0).astype(BF)

    def regroup(es):
        b64 = (lane128 & 64) != 0
        b32 = (lane128 & 32) != 0
        ys = [jnp.where(b64, es[t ^ 2], es[t]) for t in range(4)]
        return [jnp.where(b32, ys[j ^ 1], ys[j]) for j in range(4)]

    def qk_phase(g, jb, base, sl):
        pc = pieces(0, g, jb * 128)
        tri32 = row32 <= (lane32 & 31)
        klo = k_scr[g, pl.ds(base - 256, 128), :]
        kmid = k_scr[g, pl.ds(base - 128, 128), :]
        khi = k_scr[g, pl.ds(base, 128), :]
        es = []
        for t in range(4):
            lhs = jnp.concatenate([klo[32 * t:128], khi[0:32 * (t + 1)]], axis=0)
            r = lax.dot_general(lhs, group_tile(pc, t), NT, preferred_element_type=F32)
            nlo = 128 - 32 * t
            ch = []
            for c in range(4):
                if c > t:
                    ch.append(r[32 * (c - t):32 * (c - t) + 32])
                elif c < t:
                    ch.append(r[nlo + 32 * c:nlo + 32 * c + 32])
                else:
                    ch.append(jnp.where(tri32, r[nlo + 32 * t:nlo + 32 * t + 32], r[0:32]))
            es.append(jnp.concatenate(ch, axis=0))
        gs = regroup(es)
        mids = lax.dot_general(kmid, head_tiles(pc), NT, preferred_element_type=F32)
        for j in range(4):
            mid = mids[:, 128 * j:128 * (j + 1)]
            m = jnp.max(jnp.maximum(_colmax(gs[j]), _colmax(mid)), axis=0, keepdims=True)
            s_scr[sl, j, 0:128, :] = gs[j]
            s_scr[sl, j, 128:256, :] = mid
            m_scr[sl, j] = jnp.broadcast_to(m, (8, 128))

    def normalize(r):
        inv = 1.0 / r[24:32]
        return r[0:24] * jnp.concatenate([inv] * 3, axis=0)

    def finish_block(jb):
        qoff = jb * 128
        feat = lax.broadcasted_iota(jnp.int32, (32, D), 1)
        hq = ((feat * 3277) >> 16) & 3
        hb1 = (hq & 2) != 0
        hb0 = (hq & 1) != 0
        t = zt_scr[:, qoff:qoff + 128].T
        ts = [t[32 * u:32 * u + 32] for u in range(4)]
        us = [jnp.where(hb1, ts[u ^ 2], ts[u]) for u in range(4)]
        for u in range(4):
            o = jnp.where(hb0, us[u ^ 1], us[u])
            att_scr[qoff + 32 * u:qoff + 32 * u + 32, :] = o.astype(BF)

    def finish_heads(g, jb, rs):
        qoff = jb * 128
        row8 = lax.broadcasted_iota(jnp.int32, (8, 128), 0)
        for p in range(2):
            re_, ro = rs[2 * p], rs[2 * p + 1]
            z = jnp.concatenate([re_[0:16], jnp.where(row8 < 4, re_[16:24], ro[0:8]), ro[8:24]], axis=0)
            r0 = g * QW + p * 40
            zt_scr[r0:r0 + 40, qoff:qoff + 128] = z
        if g == NQUAD - 1:
            finish_block(jb)

    def pv_phase(g, jb, base, sl):
        rs = []
        for j in range(4):
            m = m_scr[sl, j][0:1, :]
            pg = jnp.exp2(s_scr[sl, j, 0:128, :] - m)
            pm = jnp.exp2(s_scr[sl, j, 128:256, :] - m)
            mhi = row128 <= (lane128 ^ (32 * j))
            phi = jnp.where(mhi, pg, 0.0)
            plo = jnp.where(mhi, 0.0, pg)
            pf = jnp.concatenate([plo, pm, phi], axis=0).astype(BF)
            vv = vt_scr[4 * g + j, :, pl.ds(base - 256, 384)]
            rs.append(normalize(jnp.dot(vv, pf, preferred_element_type=F32)))
        finish_heads(g, jb, rs)

    def qk_phase0(g, jb):
        qoff = jb * 128
        sl = jb * NQUAD + g
        pc = pieces(1, g, qoff)
        tri32 = row32 <= (lane32 & 31)
        neg32 = jnp.full((32, 128), NEG, F32)
        khi = k_scr[g, qoff:qoff + 128, :]
        es = []
        for t in range(4):
            r = lax.dot_general(khi[0:32 * (t + 1)], group_tile(pc, t), NT, preferred_element_type=F32)
            ch = [r[32 * c:32 * c + 32] for c in range(t)]
            ch.append(jnp.where(tri32, r[32 * t:32 * t + 32], NEG))
            ch += [neg32] * (3 - t)
            es.append(jnp.concatenate(ch, axis=0))
        gs = regroup(es)
        if jb > 0:
            mids = lax.dot_general(k_scr[g, 0:128, :], head_tiles(pc), NT, preferred_element_type=F32)
        for j in range(4):
            m8 = _colmax(gs[j])
            s_scr[sl, j, 0:128, :] = gs[j]
            if jb > 0:
                mid = mids[:, 128 * j:128 * (j + 1)]
                m8 = jnp.maximum(m8, _colmax(mid))
                s_scr[sl, j, 128:256, :] = mid
            m = jnp.max(m8, axis=0, keepdims=True)
            m_scr[sl, j] = jnp.broadcast_to(m, (8, 128))

    def pv_phase0(g, jb):
        nk = jb * 128 + 128
        sl = jb * NQUAD + g
        rs = []
        for j in range(4):
            m = m_scr[sl, j][0:1, :]
            phi = jnp.exp2(s_scr[sl, j, 0:128, :] - m)
            if nk > 128:
                pm = jnp.exp2(s_scr[sl, j, 128:256, :] - m)
                pf = jnp.concatenate([pm, phi], axis=0).astype(BF)
            else:
                pf = phi.astype(BF)
            rs.append(normalize(jnp.dot(vt_scr[4 * g + j, :, 0:nk], pf, preferred_element_type=F32)))
        finish_heads(g, jb, rs)

    work = [(g, jb) for jb in range(TQ // 128) for g in range(NQUAD)]

    def attention(row0, fillers):
        def base_of(jb):
            return pl.multiple_of(row0 + jb * 128, 128)

        def do_qk(n):
            g, jb = work[n]
            qk_phase(g, jb, base_of(jb), n % 2)

        nw = len(work)
        nf = len(fillers) - TAILF
        fi = 0
        do_qk(0)
        for n in range(nw):
            if n + 1 < nw:
                do_qk(n + 1)
            while fi < ((n + 1) * nf) // nw:
                fillers[fi]()
                fi += 1
            g, jb = work[n]
            pv_phase(g, jb, base_of(jb), n % 2)
        while fi < len(fillers):
            fillers[fi]()
            fi += 1

    def out_proj(prow0, r0, nr):
        xp = x_scr[pl.ds(prow0 + r0, nr), :].astype(F32)
        return xp + jnp.dot(att_scr[r0:r0 + nr, :], wo_ref[...], preferred_element_type=F32)

    def ffn_fillers(h, hn, prow0, r0, nr):
        gl = []
        fl = []
        bias = {}

        def f1(c):
            def run():
                if c == 0:
                    bias['b1'] = b1_ref[...].astype(F32).reshape(1, F)
                u = jnp.dot(hn, w1_ref[:, c * F1C:(c + 1) * F1C], preferred_element_type=F32)
                u = u + bias['b1'][:, c * F1C:(c + 1) * F1C]
                gl.append(_gelu(u).astype(BF))
            return run

        def f2(n, r):
            def run():
                if n == 0 and r == 0:
                    bias['b2'] = b2_ref[...].astype(F32).reshape(1, D)
                rows = slice(r * F2R, (r + 1) * F2R)
                cols = slice(n * 128, (n + 1) * 128)
                y = h[rows, cols] + bias['b2'][:, cols]
                for c in range(F // F1C):
                    y = y + jnp.dot(gl[c][rows], w2_ref[c * F1C:(c + 1) * F1C, cols],
                                    preferred_element_type=F32)
                o_scr[pl.ds(prow0 + (r0 + r * F2R), F2R), cols] = y.astype(BF)
            return run

        for c in range(F // F1C):
            fl.append(f1(c))
        for r in range(nr // F2R):
            for n in range(D // 128):
                fl.append(f2(n, r))
        return fl

    @pl.when(i == 0)
    def _head():
        cp_x0.start()
        cp_qk(0).start()
        cp_qk(1).start()
        cp_x0.wait()
        xn0 = ln1(0)
        qk = None
        for c in range(3):
            cp_qk(c).wait()
            if c == 0:
                cp_qk(2).start()
            elif c == 1:
                cp_x1.start()
                cp_wv.start()
            else:
                cp_wo.start()
                cp_b1.start()
                cp_b2.start()
            wc = wqkv_ref[KOFF[c]:KOFF[c + 1], 0:2 * D]
            if c == 0:
                part = jnp.concatenate(
                    [jnp.dot(xn0[r:r + 128, KOFF[c]:KOFF[c + 1]], wc, preferred_element_type=F32)
                     for r in range(0, TQ, 128)], axis=0)
            else:
                part = jnp.dot(xn0[:, KOFF[c]:KOFF[c + 1]], wc, preferred_element_type=F32)
            qk = part if qk is None else qk + part
        store_qk(_split128(qk), 0, 1)
        for g in range(NQUAD):
            qk_phase0(g, 0)
        parts = []
        st = {}
        fl = []
        for op in HSEQ.split():
            if op == 'P':
                c = len(parts)
                parts.append(jnp.dot(st['xn1'], wqkv_ref[:, c * 128:(c + 1) * 128],
                                     preferred_element_type=F32))
                if c == 9:
                    store_qk(parts, TQ, 0)
            elif op == 'W':
                cp_x1.wait()
                cp_wv.wait()
                cp_w1.start()
                cp_w2.start()
                wvt_scr[...] = wqkv_ref[:, 2 * D:3 * D].astype(F32).T.astype(BF)
                st['xn1'] = ln1(TQ)
            elif op == 'X':
                cp_wo.wait()
                cp_b1.wait()
                cp_b2.wait()
                cp_w1.wait()
                cp_w2.wait()
                cp_xr.start()
            elif op == 'Va':
                v_proj(xn0, 0, 0, H // 2)
            elif op == 'Vb':
                v_proj(xn0, 0, H // 2, H)
            elif op[0] == 'U':
                u = int(op[1])
                v_proj(st['xn1'], TQ, u * 8, u * 8 + 8)
            elif op == 'O0':
                st['h0'] = out_proj(0, 0, 128)
            elif op == 'O1':
                h = jnp.concatenate([st['h0'], out_proj(0, 128, 128)], axis=0)
                fl = ffn_fillers(h, _ln(h).astype(BF), 0, 0, TQ)
            elif op == 'F':
                fl.pop(0)()
            elif op[0] == 'q':
                qk_phase0(int(op[1]), 1)
            elif op[0] == 'a':
                pv_phase0(int(op[1]), 0)
            elif op[0] == 'b':
                pv_phase0(int(op[1]), 1)
            elif op[0] == 'K':
                n = int(op[1:])
                qk_phase(work[n][0], work[n][1], TQ + work[n][1] * 128, n % 2)
            elif op[0] == 'Z':
                n = int(op[1:])
                pv_phase(work[n][0], work[n][1], TQ + work[n][1] * 128, n % 2)
        assert len(parts) == 10 and not fl
        cp_o(0).start()
        cp_xr.wait()

    @pl.when(jnp.logical_and(i > 0, i < NSTEP - 1))
    def _main():
        row0 = pl.multiple_of((i + 1) * TQ, TQ)
        h = out_proj(row0 - TQ, 0, TQ)
        hn = _ln(h).astype(BF)
        xn = ln1(row0)
        qk = jnp.dot(xn, wqkv_ref[:, 0:2 * D], preferred_element_type=F32)
        store_qk(_split128(qk), row0, 0)
        v_proj(xn, row0, 0, H)
        attention(row0, ffn_fillers(h, hn, row0 - TQ, 0, TQ))
        cp_o(i).start()

    @pl.when(i == NSTEP - 1)
    def _last():
        prow0 = (NSTEP - 1) * TQ
        hr = TQ // 2
        ha = out_proj(prow0, 0, hr)
        hna = _ln(ha).astype(BF)
        hb = out_proj(prow0, hr, hr)
        hnb = _ln(hb).astype(BF)
        fa = ffn_fillers(ha, hna, prow0, 0, hr)
        fb = ffn_fillers(hb, hnb, prow0, hr, hr)
        n1 = F // F1C
        for f in fa[:n1] + fb[:n1] + fa[n1:] + fb[n1:n1 + 2]:
            f()
        cp_ol(0, 0, D).start()
        for f in fb[n1 + 2:n1 + 4]:
            f()
        cp_ol(1, 0, 256).start()
        for f in fb[n1 + 4:]:
            f()
        cp_ol(1, 256, D).start()
        for n in range(NSTEP - 1):
            cp_o(n).wait()
        cp_ol(0, 0, D).wait()
        cp_ol(1, 0, 256).wait()
        cp_ol(1, 256, D).wait()


@jax.jit
def pallas_sequential_preLN__sliding_block__dense_activation_gelu__prompt_kernel(
    A_x: jax.Array,
    A_wqkv: jax.Array,
    A_wo: jax.Array,
    B_x: jax.Array,
    B_w1: jax.Array,
    B_b1: jax.Array,
    B_w2: jax.Array,
    B_b2: jax.Array,
):
    del B_x
    anyspec = pl.BlockSpec(memory_space=pl.ANY)
    out = pl.pallas_call(
        _kernel,
        grid=(NSTEP,),
        in_specs=[anyspec] * 7,
        out_specs=anyspec,
        out_shape=jax.ShapeDtypeStruct((S, D), BF),
        scratch_shapes=[
            pltpu.VMEM((S, D), BF),
            pltpu.VMEM((S, D), BF),
            pltpu.VMEM((D, D), BF),
            pltpu.VMEM((2, NQUAD, TQ, 128), F32),
            pltpu.VMEM((NQUAD, S, 128), BF),
            pltpu.VMEM((H, VROWS, S), BF),
            pltpu.VMEM((TQ, D), BF),
            pltpu.VMEM((2 * NQUAD, 4, 256, 128), F32),
            pltpu.VMEM((2 * NQUAD, 4, 8, 128), F32),
            pltpu.VMEM((D, TQ), F32),
            pltpu.VMEM((D, 3 * D), BF),
            pltpu.VMEM((D, D), BF),
            pltpu.VMEM((D, F), BF),
            pltpu.VMEM((F, D), BF),
            pltpu.VMEM((F,), BF),
            pltpu.VMEM((D,), BF),
            pltpu.SemaphoreType.DMA((4,)),
        ],
        compiler_params=pltpu.CompilerParams(
            dimension_semantics=("arbitrary",),
            vmem_limit_bytes=100 * 1024 * 1024),
    )(A_x.reshape(S, D), A_wqkv, A_wo, B_w1, B_b1, B_w2, B_b2)
    return out.reshape(1, S, D)
```
